```python
import jax
import jax.numpy as jnp

def _softmax(x, axis=-1):
    return jax.nn.softmax(x, axis=axis)
def _gelu(x):
    return jax.nn.gelu(x, approximate=True)
def _silu(x):
    return jax.nn.silu(x)
def _sigmoid(x):
    return jax.nn.sigmoid(x)
def _layernorm(x, axis=-1, eps=1e-5):
    m = jnp.mean(x, axis=axis, keepdims=True)
    v = jnp.var(x, axis=axis, keepdims=True)
    return (x - m) / jnp.sqrt(v + eps)
def _scatter_add(tgt, idx, src, axis=0):
    return tgt.at[idx].add(src)
def _segment_sum(src, seg, n):
    return jax.ops.segment_sum(src, seg, n)
class _Rng:
    def __init__(self, key):
        self._k = key
    def _next(self):
        self._k, sub = jax.random.split(self._k)
        return sub
    def normal(self, shape):
        return jax.random.normal(self._next(), shape, dtype=jnp.bfloat16)
    def randint(self, lo, hi, shape):
        return jax.random.randint(self._next(), shape, lo, hi, dtype=jnp.int32)
    def uniform(self, shape, lo=0.0, hi=1.0):
        return jax.random.uniform(self._next(), shape, jnp.bfloat16, lo, hi)
    def permutation(self, n):
        return jax.random.permutation(self._next(), n)


kernel_name = 'sequential_preLN__spectral_gfnet__swiglu_ffn__prompt'

def _fwd_setup_inputs():
    _rng = _Rng(jax.random.key(int.from_bytes(__import__("os").urandom(4), "little")))
    _w = (lambda a: (lambda t: t.astype(jnp.bfloat16) if jnp.issubdtype(t.dtype, jnp.floating) else t)(jnp.asarray(a)))
    def _A_setup():
        B, S, D = 1, 2048, 576
        Df = D // 2 + 1
        return {
            "x": _w((lambda *s: _rng.normal(s) * 0.05)(B, S, D)),
            "w_r": _w((lambda *s: _rng.normal(s) * 0.05)(S, Df) * 0.02),
            "w_i": _w((lambda *s: _rng.normal(s) * 0.05)(S, Df) * 0.02),
        }
    _A_in = _A_setup()

    def _B_setup():
        B, S, D, F = 1, 2048, 576, 4608
        return {
            "x": _w((lambda *s: _rng.normal(s) * 0.05)(B, S, D)),
            "w_gate": _w((lambda *s: _rng.normal(s) * 0.05)(D, F)),
            "w_up": _w((lambda *s: _rng.normal(s) * 0.05)(D, F)),
            "w_down": _w((lambda *s: _rng.normal(s) * 0.05)(F, D)),
        }
    _B_in = _B_setup()

    return {
        "A_x": _A_in["x"],
        "A_w_r": _A_in["w_r"],
        "A_w_i": _A_in["w_i"],
        "B_x": _B_in["x"],
        "B_w_gate": _B_in["w_gate"],
        "B_w_up": _B_in["w_up"],
        "B_w_down": _B_in["w_down"],
    }

def _fwd_reference(A_x, A_w_r, A_w_i, B_x, B_w_gate, B_w_up, B_w_down):
    def _A_ref(x, w_r, w_i):
        B, S, D = x.shape
        X = (lambda x, axes=(-2,-1): jnp.fft.rfft2(x.astype(jnp.float32), axes=axes))(x, axes=(-2, -1))
        W = w_r + 1j * w_i
        X = X * W
        y = (lambda x, s, axes=(-2,-1): jnp.fft.irfft2(x, s=s, axes=axes).astype(jnp.bfloat16))(X, (S, D), axes=(-2, -1))
        return y

    def _B_ref(x, w_gate, w_up, w_down):
        g = _silu(x @ w_gate)
        u = x @ w_up
        return (g * u) @ w_down

    x = A_x
    h = x + _A_ref(_layernorm(x, axis=-1), A_w_r, A_w_i)
    h2 = h + _B_ref(_layernorm(h, axis=-1), B_w_gate, B_w_up, B_w_down)
    return h2


def setup_inputs():
    _inp = _fwd_setup_inputs()
    _gk = jax.random.fold_in(jax.random.key(int.from_bytes(__import__("os").urandom(4), "little")), 2**31 - 1)
    _shapes = [[1, 2048, 576]]
    _dtypes = ['bfloat16']
    _gks = jax.random.split(_gk, len(_shapes))
    _gs = [jax.random.normal(k, s, dtype=jnp.dtype(d)) * 0.05 for k, s, d in zip(_gks, _shapes, _dtypes)]
    _inp["grad_out"] = _gs[0]
    return _inp

def reference(A_x, A_w_r, A_w_i, B_w_gate, B_w_up, B_w_down, B_x, grad_out):
    _const = dict(B_x=B_x)
    def _f(*_d):
        return _fwd_reference(**{'A_x': _d[0], 'A_w_r': _d[1], 'A_w_i': _d[2], 'B_w_gate': _d[3], 'B_w_up': _d[4], 'B_w_down': _d[5], **_const})
    _out, _vjp = jax.vjp(_f, A_x, A_w_r, A_w_i, B_w_gate, B_w_up, B_w_down)
    _grads = _vjp(grad_out)
    _out0 = jnp.asarray(_out)
    return (_out0, *[jnp.asarray(_g) for _g in _grads])
```

```python
import numpy as np
import jax
import jax.numpy as jnp
from jax import lax
import jax.experimental.pallas as pl
import jax.experimental.pallas.tpu as pltpu

bf16 = jnp.bfloat16
f32 = jnp.float32
u32 = jnp.uint32

S, D, DF, F = 2048, 576, 289, 4608
H, SH = D // 2, S // 2
FP = 304
R = 16
BF = 512
FQ = BF // 2
NB = F // BF
TS = 256
TQ = 128
CH = 256
EPS = 1e-5

NN = (((1,), (0,)), ((), ()))
NT = (((1,), (1,)), ((), ()))
mo_ = pl.multiple_of


def _dot(a, b, dn=NN):
    return lax.dot_general(a, b, dn, preferred_element_type=f32)


def _consts():
    p = np.arange(64)[None, :]
    m = np.arange(32)
    fwd, inv = [], []
    for c in range(1, 5):
        f = np.concatenate([9 * m + c, 9 * m + 9 - c])[:, None]
        sg = np.concatenate([np.ones(32), -np.ones(32)])[:, None]
        th = 2.0 * np.pi * ((f * p) % D) / D
        co, si = np.cos(th), np.sin(th)
        a = np.block([[co, sg * si], [-si, sg * co]])
        a = a[:, np.arange(128).reshape(2, 4, 16).transpose(1, 0, 2).ravel()]
        fwd.append(a)
        inv.append(a.T * (2.0 / (S * D)))
    f = 9 * np.arange(48)[:, None]
    ok = f < DF
    edge = (f == 0) | (f == DF - 1)
    th = 2.0 * np.pi * ((f * p) % D) / D
    co = np.where(ok, np.cos(th), 0.0)
    si = np.where(ok & ~edge, -np.sin(th), 0.0)
    cf0 = np.where(edge, 1.0, 2.0) * ok / (S * D)
    a0 = np.zeros((128, 128))
    a0[:96, :64] = np.concatenate([co, si])
    b0 = np.zeros((128, 128))
    b0[:64, :96] = np.concatenate([co * cf0, si * cf0]).T
    dm = np.stack(fwd + [a0] + inv + [b0])
    cf = np.concatenate([np.full((256, 1), 2.0 / (S * D)), cf0])
    cf = np.broadcast_to(cf, (FP, 128)).astype(np.float32)
    k1 = np.arange(R)[:, None, None]
    s2 = np.arange(128)[None, :, None]
    ln = np.arange(128)[None, None, :]
    j = (ln - k1) % R
    k = 128 * j + (ln - j) % 128
    ph = 2.0 * np.pi * ((s2 * k) % S) / S
    g = np.concatenate([np.cos(ph), np.sin(ph)], axis=1)
    tobf = lambda a: np.ascontiguousarray(a.astype(np.float32)).astype(bf16)
    return tobf(dm), tobf(g), np.ascontiguousarray(cf)


_DM, _G, _CF = _consts()
_RHO = (1, 8, 2, 7, 3, 6, 4, 5, 0)
_H3 = float(np.sqrt(3.0) / 2.0)


def _cmul(v, e, n):
    re, im = v
    e = e % n
    if e == 0:
        return re, im
    if 4 * e == n:
        return -im, re
    if 4 * e == 3 * n:
        return im, -re
    c = float(np.cos(2 * np.pi * e / n))
    s = float(np.sin(2 * np.pi * e / n))
    if (8 * e) % n == 0:
        if c * s > 0:
            return (re - im) * c, (re + im) * c
        return (re + im) * c, (im - re) * c
    return re * c - im * s, re * s + im * c


def _dft4(a, sign):
    (ar, ai), (br, bi), (cr, ci), (dr, di) = a
    pr, pi_, mr, mi = ar + cr, ai + ci, ar - cr, ai - ci
    qr, qi, nr, ni = br + dr, bi + di, br - dr, bi - di
    o1 = (mr - ni, mi + nr)
    o3 = (mr + ni, mi - nr)
    if sign < 0:
        o1, o3 = o3, o1
    return [(pr + qr, pi_ + qi), o1, (pr - qr, pi_ - qi), o3]


def _dft16(v, sign):
    cols = [_dft4([v[n2 + 4 * n1] for n1 in range(4)], sign) for n2 in range(4)]
    out = [None] * 16
    for k1 in range(4):
        r = _dft4([_cmul(cols[n2][k1], sign * n2 * k1, 16) for n2 in range(4)], sign)
        for k2 in range(4):
            out[k1 + 4 * k2] = r[k2]
    return out


def _dft3(a, sign):
    (ar, ai), (br, bi), (cr, ci) = a
    sr, si = br + cr, bi + ci
    dr, di = (br - cr) * (sign * _H3), (bi - ci) * (sign * _H3)
    mr, mi = ar - 0.5 * sr, ai - 0.5 * si
    return [(ar + sr, ai + si), (mr - di, mi + dr), (mr + di, mi - dr)]


def _rdft3(a, b, c):
    s = b + c
    return a + s, (a - 0.5 * s, (c - b) * _H3)


def _irdft3(a, u):
    m = a - 0.5 * u[0]
    t = u[1] * _H3
    return [a + u[0], m - t, m + t]


def _rdft9(v):
    st = [_rdft3(v[q], v[q + 3], v[q + 6]) for q in range(3)]
    t0, t3 = _rdft3(st[0][0], st[1][0], st[2][0])
    t1, t4, t7 = _dft3([_cmul(st[q][1], -q, 9) for q in range(3)], -1)
    return t0, [t1, (t7[0], -t7[1]), t3, t4]


def _irdft9(u0, u):
    a0 = _irdft3(u0, u[2])
    b = _dft3([u[0], u[3], (u[1][0], -u[1][1])], 1)
    y = [_irdft3(a0[q], _cmul(b[q], q, 9)) for q in range(3)]
    return [y[q % 3][q // 3] for q in range(9)]


def _fold(v):
    return v[:8] + v[8:]


def _mean(acc):
    return jnp.sum(acc, axis=0, keepdims=True) * (1.0 / D)


def _acc(a, v):
    return v if a is None else a + v


def _act(g, u, da):
    sg = 0.5 * jnp.tanh(0.5 * g) + 0.5
    sl = g * sg
    return sl * u, da * u * (sg + sl * (1.0 - sg)), da * sl


def _cA(a11, a12, a21, a22):
    return [a11 + a22, a21 + a22, a11, a22, a11 + a12, a21 - a11, a12 - a22]


def _cB(b11, b12, b21, b22):
    return [b11 + b22, b11, b12 - b22, b21 - b11, b22, b11 + b12, b21 + b22]


def _cC(m):
    return (m[0] + m[3] - m[4] + m[6], m[2] + m[4], m[1] + m[3], m[0] - m[1] + m[2] + m[5])


_PERM = (0, 2, 6, 5, 3, 4, 1)


def _barrel(v, sign):
    lane = lax.broadcasted_iota(jnp.int32, v[0].shape, 1)
    for t in (1, 2, 4, 8):
        mk = (lane & t) != 0
        v = [jnp.where(mk, v[(i - sign * t) % R], v[i]) for i in range(R)]
    return v


class _Packed:
    def __init__(self, ref):
        self.ref = ref

    def _ix(self, ix):
        ix = () if ix is Ellipsis else ix if isinstance(ix, tuple) else (ix,)
        ix = list(ix) + [slice(None)] * (len(self.ref.shape) - len(ix))
        r = ix[-2]
        if isinstance(r, slice):
            ix[-2] = slice(*(None if v is None else v // 2 for v in (r.start, r.stop)))
        else:
            ix[-2] = pl.ds(mo_(r.start >> 1, 8), r.size // 2)
        return tuple(ix)

    def view(self, ix):
        return _Packed(self.ref.at[self._ix(ix)])

    def __getitem__(self, ix):
        return pltpu.bitcast(self.ref[self._ix(ix)], bf16)

    def __setitem__(self, ix, v):
        self.ref[self._ix(ix)] = pltpu.bitcast(v, u32)


_PACKED = ("hnT", "a_k", "vT", "xs", "wT", "ac", "w1", "w2", "hb", "wdl", "acl", "hc", "oc")
_ODD = ("mo", "mh", "hc", "oc", "hb", "zT", "ub", "ac", "w1", "w2", "acc", "dh", "acl", "vT", "hnT")


def _scratch(name, shape, dtype):
    if name in _ODD:
        shape = shape[:-1] + (shape[-1] + 128,)
    if name in _PACKED:
        return pltpu.VMEM(shape[:-2] + (shape[-2] // 2, shape[-1]), u32)
    return pltpu.VMEM(shape, dtype)


_SCR = dict(
    xT=((D, S), bf16), goT=((D, S), bf16), wraw=((2, DF, S), bf16),
    dm=((10, 128, 128), bf16), g=((R, 256, 128), bf16), cf=((FP, 128), f32),
    st=((8, S), f32), hnT=((D, S), bf16),
    zT=((2 * FP, S), f32), a_k=((R, FP, 256), bf16),
    vT=((2 * FP, S), bf16), xs=((R, FP, 256), bf16), wT=((R, FP, 256), bf16),
    wsc=((2 * R, FP, 128), f32), dh=((D, S), f32),
    wb=((2, 3, D, BF), bf16), ob=((2, 3, D, BF), bf16),
    ac=((7, 3 * FQ, TS), bf16),
    w1=((18 * FQ, 768), bf16), w2=((14 * H, 3 * FQ), bf16), hb=((2, 15 * 128, SH), bf16),
    wl=((D, BF), bf16), wdl=((BF, D), bf16), acl=((7, 2 * FQ, SH), bf16),
    ub=((D, S), f32), hc=((7, H, SH), bf16), oc=((7, H, SH), bf16), mo=((7, H, SH), f32), mh=((7, H, SH), f32),
    acc=((2, 7, H, 3 * FQ), f32),
)


def _kernel(x_h, go_h, wr_h, wi_h, dm_h, g_h, cf_h, wg_h, wu_h, wd_h,
            out_h, dx_h, dwr_h, dwi_h, dwg_h, dwu_h, dwd_h,
            xT, goT, wraw, dm, g_r, cf_r, st, hnT, zT, a_k, vT, xs, wT, wsc, dh,
            wb, ob, ac, w1, w2, hb, wl, wdl, acl, ub, hc, oc, mo, mh, acc, sx, sm, sw, so_):
    hnT, a_k, vT, xs, wT, ac, w1, w2, hb, wdl, acl, hc, oc = map(
        _Packed, (hnT, a_k, vT, xs, wT, ac, w1, w2, hb, wdl, acl, hc, oc))
    tb = vT
    cp = pltpu.make_async_copy
    col = lambda i, n: pl.ds(mo_(i * n, n), n)

    def x_cp(i):
        return cp(x_h.at[:, col(i, CH)], xT.at[:, col(i, CH)], sx.at[i])

    def dx_cp(i):
        return cp(xT.at[:, col(i, CH)], dx_h.at[:, col(i, CH)], sx.at[i])

    def w_cp(b, sl):
        return [cp(w.at[:, col(b, BF)], wb.at[sl, m], sw.at[sl * 3 + m])
                for m, w in enumerate((wg_h, wu_h, wd_h))]

    def o_cp(b, sl):
        return [cp(ob.at[sl, m], w.at[:, col(b, BF)], so_.at[sl * 3 + m])
                for m, w in enumerate((dwg_h, dwu_h, dwd_h))]

    c_dm = cp(dm_h, dm, sm.at[0])
    c_wr = cp(wr_h, wraw.at[0], sm.at[1])
    c_wi = cp(wi_h, wraw.at[1], sm.at[2])
    c_g = cp(g_h, g_r, sm.at[3])

    def go_cp(i):
        return [cp(go_h.at[:, col(i + 4 * e, CH)], goT.at[:, col(i + 4 * e, CH)], sx.at[i + 4 * e])
                for e in range(2)]
    c_cf = cp(cf_h, cf_r, sm.at[5])
    c_wl = cp(wd_h.at[:, F - BF:], wl, sm.at[4])
    for i in range(S // CH):
        x_cp(i).start()

    def grp(q, p):
        return slice(64 * q + 16 * p, 64 * q + 16 * p + 16)

    def d_rows(val, r):
        for p in range(4):
            t0, t = _rdft9([val(grp(q, p)) for q in range(9)])
            for c in range(4):
                for e in range(2):
                    o = 128 * c + 32 * p + 16 * e
                    tb[o:o + 16, r] = t[c][e].astype(bf16)
            tb[512 + 16 * p:528 + 16 * p, r] = t0.astype(bf16)

    def d_mm(c, scaled, r=slice(0, S)):
        m = dm[c] if c < 4 else dm[4, :96, :64]
        z = _dot(m, tb[128 * c:min(128 * c + 128, D), r])
        z = z * st[1:2, r] if scaled else z
        n = z.shape[0] // 2
        zT[64 * c:64 * c + n, r] = z[:n]
        zT[FP + 64 * c:FP + 64 * c + n, r] = z[n:]

    def i_mm(c, r):
        n = 64 if c < 4 else 48
        v = jnp.concatenate([vT[o + 64 * c:o + 64 * c + n, r] for o in (0, FP)], axis=0)
        u = _dot(dm[5 + c] if c < 4 else dm[9, :64, :96], v)
        ub[128 * c:128 * c + u.shape[0], r] = u
        return u

    def i_rows(cols, emit, pace):
        for p in range(4):
            for k, r in enumerate(cols):
                t = lambda o: ub[o:o + 16, r]
                y = _irdft9(t(512 + 16 * p), [(pace(t(128 * c + 32 * p)), pace(t(128 * c + 32 * p + 16)))
                                              for c in range(4)])
                for q in range(9):
                    emit(k, grp(q, p), y[q])

    def loop(n, fn):
        def body(i, c):
            fn(i)
            return c
        lax.fori_loop(0, n, body, 0)

    adj = lambda i: [col(2 * i, 128), col(2 * i + 1, 128)]
    far = lambda i: [col(i, 128), col(i + 8, 128)]

    def z16(i):
        ra, rb = col(i, 16), pl.ds(mo_(FP + i * 16, 16), 16)
        return ra, rb, [(zT[ra, j * 128:(j + 1) * 128], zT[rb, j * 128:(j + 1) * 128])
                        for j in range(R)]

    def fwd16(scaled):
        d_mm(4, scaled)
        for n, c in enumerate((4, 0, 1, 2, 3)):
            if n < 4:
                d_mm(n, scaled)
            for t in range(4 * c, min(4 * c + 4, FP // 16)):
                ra, _, v = z16(t)
                for k, o in enumerate(_dft16(v, -1)):
                    a_k[k, tiles[t], 0:128] = o[0].astype(bf16)
                    a_k[k, tiles[t], 128:256] = o[1].astype(bf16)

    def inv16(extra):
        def body(i):
            ra, rb, v = z16(i)
            for j, o in enumerate(_dft16(v, 1)):
                vT[ra, j * 128:(j + 1) * 128] = o[0].astype(bf16)
                vT[rb, j * 128:(j + 1) * 128] = o[1].astype(bf16)
        loop(FP // 16, body)

        def mm(i):
            for c in range(5):
                extra(i, c, i_mm(c, col(i, S // 2)))
        loop(2, mm)

    def gmat(k):
        c, s = g_r[k, :128], g_r[k, 128:]
        return jnp.concatenate([jnp.concatenate([c, -s], axis=1),
                                jnp.concatenate([s, c], axis=1)], axis=0)

    def rstart(i):
        return mo_(64 * i + jnp.where(i >= 2, 16, 0), 16)

    pieces = [(m, t) for t in range(5) for m in range(3)]

    def prep2(sl, i, m, t, tie=lambda v: v):
        r0 = rstart(i) + 16 * t
        ra, rb = pl.ds(mo_(r0, 16), 16), pl.ds(mo_(H + r0, 16), 16)
        w = lambda r, c: tie(wb[sl, m, r, c * FQ:(c + 1) * FQ].astype(f32))
        dst = w2.view(pl.ds(mo_(sl * 7 * H + r0, 16), 6 * H + 16))
        for j, v in enumerate(_cB(w(ra, 0), w(rb, 0), w(ra, 1), w(rb, 1))):
            dst[j * H:j * H + 16, m * FQ:(m + 1) * FQ] = v.astype(bf16)

    lay = {0: (0, 0, 256), 3: (0, 256, 256), 4: (0, 512, 256), 1: (1, 0, 384), 2: (1, 384, 384),
           5: (2, 0, 384), 6: (2, 384, 384)}

    def prep1(sl, i, m, part, tie_=lambda v: v):
        k0, fh = mo_((i >> 1) * 128, 128), i & 1
        src = wb.at[sl, m, :, pl.ds(mo_(fh * 128, 128), 384)]
        r0_, n_, step, o_ = (fh * 256, 1792, 32, 16 * m) if m < 2 else (512 + fh * 128, 1664, 16, 0)
        dst = w1.view((pl.ds(mo_(sl * 9 * FQ + r0_, 128), n_),
                       slice(None) if part else pl.ds(k0, 640)))
        if part == 0:
            src = src.at[pl.ds(k0, 384)]

        def ld(r0, n, o):
            return jnp.concatenate(
                [tie_(src[r0 + 16 * t:r0 + 16 * t + 16, 256 * o:256 * o + 128])
                 for t in range(n // 16)], axis=0)

        def put(j, c0, v):
            v = v.astype(bf16)
            for t in range(8):
                r0, c = lay[j][0] * 3 * FQ + step * t + o_, lay[j][1] + c0
                dst[r0:r0 + 16, c:c + 128] = v[16 * t:16 * t + 16]
        if part == 0:
            a = [ld(kk, 128, o).T.astype(f32) for o in (0, 1) for kk in (0, 256)]
            cs = _cA(*a)
            for j, v in enumerate(cs):
                put(j, 0, v)
            return cs[1].astype(bf16), cs[4].astype(bf16)
        else:
            r1, r2 = ld(512, 64, 0), ld(512, 64, 1)
            t1 = jnp.concatenate([r1, r2], axis=0).T.astype(f32)
            t2 = jnp.concatenate([r2, r1], axis=0).T.astype(f32)
            low = lax.broadcasted_iota(jnp.int32, (128, 128), 1) < 64
            put(1, 256, jnp.where(low, t2, 0.0))
            put(2, 256, jnp.where(low, 0.0, t2))
            put(5, 256, jnp.where(low, t2, t1 - t2))
            put(6, 256, jnp.where(low, t1, 0.0))
            return t1.astype(bf16), t2.astype(bf16)

    def final(sl, i, m, t, tie=lambda v: v):
        r0 = rstart(i) + 16 * t
        ra, rb = pl.ds(mo_(r0, 16), 16), pl.ds(mo_(H + r0, 16), 16)
        ms = [acc[sl, j, ra, m * FQ:(m + 1) * FQ] for j in range(7)]
        ms = [tie(v) if j in (0, 3, 4) else v for j, v in enumerate(ms)]
        c11, c12, c21, c22 = (v.astype(bf16) for v in _cC(ms))
        ob[sl, m, ra, :FQ] = c11
        ob[sl, m, ra, FQ:] = c12
        ob[sl, m, rb, :FQ] = c21
        ob[sl, m, rb, FQ:] = c22

    tiles = [slice(16 * t, 16 * t + 16) for t in range(D // 16)]

    def fill_b(n, src, t, r, r2, tie_=lambda v: v):
        if t < 16:
            c4 = [tie_(src[tiles[t + o], rr].astype(f32)) for o in (0, 16) for rr in (r, r2)]
            for j, v in enumerate(_cB(*c4)):
                hb[n, tiles[t].start + 256 * j:tiles[t].stop + 256 * j, r] = v.astype(bf16)
        else:
            for e in range(2):
                for k, rr in enumerate((r, r2)):
                    u = 2 * (t - 16) + e
                    o = 1792 + 64 * k + 16 * u
                    hb[n, o:o + 16, r] = src[tiles[32 + u], rr]

    def p1(i):
        @pl.when(i == 1)
        def _():
            c_dm.start()
            c_wr.start()
            c_wi.start()
            c_g.start()
        x_cp(i).wait()
        for r in adj(i):
            s1 = None
            for t in tiles:
                s1 = _acc(s1, _fold(xT[t, r].astype(f32)))
            m = _mean(s1)
            s2 = [None]

            def val(rows):
                v = xT[rows, r].astype(f32) - m
                s2[0] = _acc(s2[0], _fold(v * v))
                return v
            d_rows(val, r)
            st[0:1, r] = m
            st[1:2, r] = lax.rsqrt(_mean(s2[0]) + EPS)
    loop(S // CH, p1)

    c_dm.wait()
    fwd16(True)

    c_wr.wait()
    c_wi.wait()
    for c in (*go_cp(0), *go_cp(1)):
        c.start()

    def wperm(rows, load):
        for q in range(2):
            v = []
            for j in range(R):
                t = pltpu.bitcast(load(q, slice(j * 128, (j + 1) * 128)), u32)
                v.append(pltpu.roll(t, j, 1) if j else t)
            v = _barrel([v[-i % R] for i in range(R)], 1)
            for k in range(R):
                wsc[q * R + k, rows, :] = pltpu.bitcast(v[k], bf16).astype(f32)

    def pw(i, c):
        rows = col(i, 32)
        wperm(rows, lambda q, cs: wraw[q, rows, cs])
        acc[1, :, rows, :3 * FQ] = jnp.zeros((7, 32, 3 * FQ), f32)
        return c
    lax.fori_loop(0, 9, pw, 0)
    row0 = lax.broadcasted_iota(jnp.int32, (16, 128), 0) == 0
    wperm(slice(288, 304), lambda q, cs: jnp.where(
        row0, jnp.broadcast_to(wraw[q, 288:289, cs].astype(f32), (16, 128)), 0.0).astype(bf16))

    c_g.wait()

    def tie(never, z, o, w=FQ):
        return lambda v: jnp.where(never, z[o:o + 16, :w], v)

    def pacer(never, parts, n, lead=0.2):
        zs, cnt = [], [0]

        def pace(v):
            pos = (cnt[0] - lead * n) * 3.44 / ((1.0 - lead) * n)
            cnt[0] += 1
            if pos < 0:
                return v
            while len(zs) <= int(pos):
                zs.append(next(parts))
            z = zs[int(pos)]
            return tie(never, z, int((pos % 1) * z.shape[0] // 16) * 16, 128)(v)
        return pace

    def s_stage(i, mid, side):
        gm = [gmat(4 * i + e) for e in range(4)]
        X = [_dot(a_k[4 * i], gm[0])]
        for e in range(4):
            k = 4 * i + e
            if e < 3:
                X.append(_dot(a_k[k + 1], gm[e + 1]))
                side(X[-1])
            B = _dot(mid(k, X[e]).astype(bf16), gm[e], NT)
            zT[:FP, col(k, 128)] = B[:, :128]
            zT[FP:, col(k, 128)] = B[:, 128:]
            if e < 3:
                side(B)

    def p3k(k, X):
        xs[k] = X.astype(bf16)
        wr, wi = (jnp.concatenate([wsc[q * R + k, pl.ds(p, 32, stride=9), :] for p in _RHO]
                                  + [wsc[q * R + k, 288:304, :]], axis=0) for q in range(2))
        wT[k] = jnp.concatenate([wr, wi], axis=1).astype(bf16)
        xr, xi = X[:, :128], X[:, 128:]
        return jnp.concatenate([xr * wr - xi * wi, xr * wi + xi * wr], axis=1)

    def p3(i, c):
        @pl.when(i == 0)
        def _():
            for c_ in (*go_cp(2), *go_cp(3)):
                c_.start()

        @pl.when(i == 2)
        def _():
            for c_ in w_cp(0, 0):
                c_.start()
        for c_ in go_cp(i):
            c_.wait()
        r, r2 = col(i, CH), col(i + 4, CH)
        todo = list(tiles[:H // 16])

        def side(z):
            for o in (0, 96, 192):
                t = todo.pop()
                g4 = [tie(i < 0, z, o)(goT[h + t.start:h + t.stop, rr].astype(f32))
                      for h in (0, H) for rr in (r, r2)]
                for j, v in enumerate(_cA(*g4)):
                    oc[j, t, r] = v.astype(bf16)
                fill_b(1, goT, t.start // 16, r, r2, tie(i < 0, z, o))
                for j in (0, 3, 4):
                    mo[j, t, r] = tie(i < 0, z, o)(jnp.zeros((16, CH), f32))
        s_stage(i, p3k, side)
        return c
    lax.fori_loop(0, 4, p3, 0)
    for c in w_cp(0, 0):
        c.wait()
    for c in (c_wl, c_cf):
        c.start()

    def prep0(i, c, z):
        for e in range(2):
            for m in range(3):
                prep2(0, 2 * i + e, m, c, tie(i < 0, z, 16 * m))
            if c < 3:
                for part in range(2):
                    prep1(0, 2 * i + e, c, part, tie(i < 0, z.astype(bf16), 64 * e + 32 * part, 128))
    inv16(prep0)
    c_wl.wait()
    for c in w_cp(1, 1):
        c.start()

    def pl_(i):
        wt = wl[:, col(i, 128)].T
        for t in range(8):
            wdl[col(2 * ((i & 1) * 8 + t) + (i >> 1), 16), :] = wt[16 * t:16 * t + 16]
    loop(4, pl_)

    def p5(i):
        cols = far(i)
        r = cols[0]
        slot = ((6, 2), (1, 5))

        def href(k, rows):
            hf = rows.start // H
            return mo.at[slot[k][hf], rows.start - hf * H:rows.stop - hf * H, r]
        s1 = [None, None]

        def early_da():
            for c_ in cols:
                da = _dot(wdl[...], goT[:, c_])
                dh[:BF, c_] = da
                yield da[:FQ]
                yield da[FQ:]
        pace = pacer(i < 0, early_da(), 64 + 54)

        def emit(k, rows, y):
            h = xT[rows, cols[k]].astype(f32) + y
            href(k, rows)[...] = h
            s1[k] = _acc(s1[k], _fold(h))
        i_rows(cols, emit, pace)
        m, rstd = [], []
        for k in range(2):
            m.append(_mean(s1[k]))
            s2 = None
            for t in tiles:
                v = href(k, t)[...] - m[k]
                s2 = _acc(s2, _fold(v * v))
            rstd.append(lax.rsqrt(_mean(s2) + EPS))
            st[2:3, cols[k]] = rstd[k]
        for t in tiles[:H // 16]:
            h11, h21, h12, h22 = mo[6, t, r], pace(mo[1, t, r]), pace(mo[2, t, r]), pace(mo[5, t, r])
            mo[5, t, r] = h22 - h12 + h21
            n = [(v - m[k]) * rstd[k] for v, k in ((h11, 0), (h21, 1), (h12, 0), (h22, 1))]
            cs = [v.astype(bf16) for v in _cA(*n)]
            t2 = slice(H + t.start, H + t.stop)
            hnT[t, cols[0]] = cs[2]
            hnT[t, cols[1]] = n[1].astype(bf16)
            hnT[t2, cols[0]] = n[2].astype(bf16)
            hnT[t2, cols[1]] = cs[3]
            for j, v in enumerate(cs):
                hc[j, t, r] = v
    loop(8, p5)
    loop(4, lambda i: [fill_b(0, hnT, t, col(i, CH), col(i + 4, CH)) for t in range(18)])


    def ffn(b, sl, so, last):
        def body(i, c):
            r = col(i, TS)
            nv = i < 0
            w1v = w1.view(pl.ds(sl * 9 * FQ if last else mo_(sl * 9 * FQ, 128), 9 * FQ))
            w2v = w2.view(pl.ds(sl * 7 * H if last else mo_(sl * 7 * H, 16), 7 * H))
            tok = lambda hf, q: pl.ds(mo_(hf * SH + i * TS + q * TQ, TQ), TQ)

            def park(q, j, n, o, nr):
                return (zT, ub)[q].at[o:o + nr, (2 * j + n) * 128:(2 * j + n + 1) * 128]

            def elem(q, t, tie_):
                c = []
                for n, o in ((0, 32 * t), (0, 32 * t + 16), (1, 16 * t)):
                    if n == 1 and last:
                        c.append([dh[32 * t + 16 * fh:32 * t + 16 * fh + 16, tok(hf, q)]
                                  for fh in range(2) for hf in range(2)])
                    else:
                        ms = [park(q, j, n, o, 16)[...] for j in range(7)]
                        c.append(_cC([tie_(v) if j in (0, 3, 4) else v for j, v in enumerate(ms)]))
                p = [_act(c[0][n], c[1][n], c[2][n]) for n in (0, 2, 1, 3)]
                for m, n in enumerate((1, 2, 0)):
                    for j, v in enumerate(_cA(*(e[n] for e in p))):
                        ac[j, m * FQ + 16 * t:m * FQ + 16 * t + 16, q * TQ:(q + 1) * TQ] = v.astype(bf16)

            def drain(todo, fn, z, n, w):
                for e in range(n):
                    if todo:
                        fn(todo.pop(0), tie(nv, z, z.shape[0] * e // n // 16 * 16, w))

            def s1(q, todo, fn, cnt):
                for n, o, nr in ((1, 2 * FQ, FQ), (0, 0, 2 * FQ))[int(last):]:
                    for j in range(7):
                        pn, c0, kk = lay[j]
                        rhs = hb[n, 256 * j:256 * j + 256, tok(0, q)]
                        if kk > 256:
                            rhs = jnp.concatenate([rhs, hb[n, 1792:, tok(0, q)]], axis=0)
                        z = _dot(w1v[pn * 3 * FQ + o:pn * 3 * FQ + o + nr, c0:c0 + kk], rhs)
                        park(q, j, n, 0, nr)[...] = z
                        drain(todo, fn, z, cnt[n], TQ)

            prev = [None]

            def s2(q, todo, fn, cnt, before=()):
                done = []
                qs = slice(q * TQ, (q + 1) * TQ)
                for j in range(7):
                    wr_ = slice(j * H, (j + 1) * H)
                    rhs = ac[j, :2 * FQ, qs]
                    if 1 <= j <= len(before):
                        v0, v1 = done[j - 1]
                        rhs = jnp.concatenate([jnp.where(nv, v0, rhs[:128]),
                                               jnp.where(nv, v1, rhs[128:256]), rhs[256:]], axis=0)
                    if j < len(before):
                        done.append(prep1(so, i, *before[j], tie(nv, prev[0].astype(bf16), 128, TQ)))
                    z = _dot(w2v[wr_, :2 * FQ], rhs)
                    prev[0] = z
                    mh[j, :, tok(0, q)] = jnp.where(b == 0, 0.0, mh[j, :, tok(0, q)]) + z
                    drain(todo, fn, z, cnt[0], TQ)
                    z = _dot(w2v[wr_, 2 * FQ:3 * FQ], ac[j, 2 * FQ:, qs])
                    mo[j, :, tok(0, q)] += z
                    drain(todo, fn, z, cnt[1], TQ)

            wide = lambda tie_: lambda v: jnp.concatenate([tie_(v[:, :TQ]), tie_(v[:, TQ:])], axis=1)
            s1(0, list(pieces), lambda p, t_: final(so, i, *p, wide(t_)), (3 if last else 2, 1))
            rest = list(range(16))
            s1(1, rest, lambda t, t_: elem(0, t, t_), (2, 1))
            for t in rest:
                elem(0, t, lambda v: v)
            s2(0, list(range(16)), lambda t, t_: elem(1, t, t_), (2, 1))
            s2(1, [], None, (0, 0), [] if last else [(m, p) for m in range(3) for p in range(2)])
            todo = list(pieces)
            for j in range(7):
                if last:
                    acl[j, :, r] = ac[_PERM[j], :2 * FQ, :TS]
                else:
                    z = _dot(hc[j, :, r], ac[_PERM[j], :2 * FQ, :TS], NT)
                    acc[sl, j, :, :2 * FQ] = jnp.where(i == 0, 0.0, acc[sl, j, :, :2 * FQ]) + z
                    drain(todo, lambda p, t_: prep2(so, i, *p, t_), z, 3 - (j > 0), FQ)
                acc[sl, j, :, 2 * FQ:3 * FQ] = jnp.where(i == 0, 0.0, acc[sl, j, :, 2 * FQ:3 * FQ]) + _dot(
                    oc[j, :, r], ac[_PERM[j], 2 * FQ:, :TS], NT)
            return c
        return body

    def block(b, c):
        sl = b & 1
        so = 1 - sl

        for c_ in w_cp(b + 1, so):
            c_.wait()

        @pl.when(b + 2 < NB)
        def _():
            for c_ in w_cp(b + 2, sl):
                c_.start()

        @pl.when(b >= 3)
        def _():
            for c_ in o_cp(b - 3, so):
                c_.wait()

        lax.fori_loop(0, SH // TS, ffn(b, sl, so, False), 0)

        @pl.when(b >= 1)
        def _():
            for c_ in o_cp(b - 1, so):
                c_.start()
        return c
    lax.fori_loop(0, NB - 1, block, 0)
    ls = (NB - 1) % 2
    for c in o_cp(NB - 4, 1 - ls):
        c.wait()
    lax.fori_loop(0, SH // TS, ffn(NB - 1, ls, 1 - ls, True), 0)
    for c in o_cp(NB - 2, 1 - ls):
        c.start()

    for c in o_cp(NB - 3, ls):
        c.wait()

    def flush(m):
        loop(4, lambda i: [final(ls, i, m, t) for t in range(5)])
        o_cp(NB - 1, ls)[m].start()

    def late_dw(m, i):
        j = jnp.minimum(i, 6)
        for o in (m * FQ, m * FQ + 128):
            z0 = _dot(hc[j, :, :512], acl[j, o:o + 128, :512], NT)
            yield z0
            z1 = _dot(hc[j, :, 512:SH], acl[j, o:o + 128, 512:SH], NT)
            acc[ls, j, :, o:o + 128] = z0 + z1
            yield z1
    flush(2)

    def e1(i):
        pace = pacer(i < 0, late_dw(0, i), 18 + 72, 0.07)
        cols = far(i)
        r = cols[0]
        s1, s2 = [None, None], [None, None]
        for t in tiles[:H // 16]:
            t2 = slice(H + t.start, H + t.stop)
            cc = _cC([pace(mh[0, t, r])] + [mh[j, t, r] for j in range(1, 7)])
            for dn, k, rows in zip(cc, (0, 0, 1, 1), (t, t2, t, t2)):
                dh[rows, cols[k]] = dn
                s1[k] = _acc(s1[k], _fold(dn))
                s2[k] = _acc(s2[k], _fold(dn * hnT[rows, cols[k]].astype(f32)))
        for k, rr in enumerate(cols):
            m1, m2, rstd = _mean(s1[k]), _mean(s2[k]), st[2:3, rr]

            def val(rows):
                v = goT[rows, rr].astype(f32) + (
                    pace(dh[rows, rr]) - m1 - hnT[rows, rr].astype(f32) * m2) * rstd
                dh[rows, rr] = v
                return v
            d_rows(val, rr)
    loop(8, e1)
    flush(0)
    fwd16(False)
    c_cf.wait()

    def e3k(k, G):
        gr, gi = G[:, :128], G[:, 128:]
        X = xs[k].astype(f32)
        xr, xi = X[:, :128], X[:, 128:]
        cf = cf_r[...]
        for q, dw in enumerate(((gr * xr + gi * xi) * cf, (gi * xr - gr * xi) * cf)):
            for n, p in enumerate(_RHO):
                wsc[q * R + k, pl.ds(p, 32, stride=9), :] = dw[32 * n:32 * n + 32]
            wsc[q * R + k, 288:304, :] = dw[288:]
        w = wT[k].astype(f32)
        wr, wi = w[:, :128], w[:, 128:]
        return jnp.concatenate([gr * wr + gi * wi, gi * wr - gr * wi], axis=1)

    def e3(i, c):
        r, r2 = col(i, CH), col(i + 4, CH)
        todo = list(tiles[:H // 16])

        def side(z):
            for o in (0, 96, 192):
                t = todo.pop()
                t2 = slice(H + t.start, H + t.stop)
                ms = [mo[j, t, r] for j in range(7)]
                cc = _cC([tie(i < 0, z, o)(v) if j in (0, 3, 4) else v for j, v in enumerate(ms)])
                for v, rr, rows in zip(cc, (r, r, r2, r2), (t, t2, t, t2)):
                    goT[rows, rr] = v.astype(bf16)
        s_stage(i, e3k, side)
        return c
    lax.fori_loop(0, 4, e3, 0)
    c_out = cp(goT, out_h, sm.at[4])
    c_out.start()

    def wunperm(rows, store, tie_=lambda v: v):
        for q in range(2):
            v = _barrel([pltpu.bitcast(tie_(wsc[q * R + k, rows, :]).astype(bf16), u32)
                         for k in range(R)], -1)
            for j in range(R):
                t = v[-j % R]
                t = pltpu.roll(t, 128 - j, 1) if j else t
                store(q, slice(j * 128, (j + 1) * 128), pltpu.bitcast(t, bf16))

    def ew(i, c, z):
        for n in range(3 * c, min(3 * c + 3, 9)):
            rows = col(9 * i + n, 16)

            def store(q, cs, t):
                wraw[q, rows, cs] = t
            wunperm(rows, store, tie(i < 0, z, 32 * (n % 3), 128))

    def store_last(q, cs, t):
        wraw[q, 288:289, cs] = t.astype(f32)[0:1].astype(bf16)
    wunperm(slice(288, 304), store_last)
    inv16(ew)
    c_dwr = cp(wraw.at[0], dwr_h, sm.at[1])
    c_dwi = cp(wraw.at[1], dwi_h, sm.at[2])
    c_dwr.start()
    c_dwi.start()

    def e5(i):
        pace = pacer(i < 0, late_dw(1, i), 16 * 4 + 36)
        cols = adj(i)
        m = [st[0:1, r] for r in cols]
        rstd = [st[1:2, r] for r in cols]
        s1, s2 = [None, None], [None, None]

        def emit(k, rows, dn):
            zT[rows, cols[k]] = dn
            s1[k] = _acc(s1[k], _fold(dn))
            s2[k] = _acc(s2[k], _fold(dn * (xT[rows, cols[k]].astype(f32) - m[k])))
        i_rows(cols, emit, pace)
        for k, r in enumerate(cols):
            m1 = _mean(s1[k])
            m2 = _mean(s2[k]) * rstd[k] * rstd[k]
            for t in tiles:
                cx = xT[t, r].astype(f32)
                cx = (pace(cx) if t.start % 32 == 0 else cx) - m[k]
                xT[t, r] = (dh[t, r] + (zT[t, r] - m1 - cx * m2) * rstd[k]).astype(bf16)
        dx_cp(i).start()
    loop(S // CH, e5)
    flush(1)

    for c in (*o_cp(NB - 2, 1 - ls), *o_cp(NB - 1, ls), c_out, c_dwr, c_dwi):
        c.wait()
    for i in range(S // CH):
        dx_cp(i).wait()


@jax.jit
def pallas_sequential_preLN__spectral_gfnet__swiglu_ffn__prompt_kernel(
    A_x: jax.Array,
    A_w_r: jax.Array,
    A_w_i: jax.Array,
    B_x: jax.Array,
    B_w_gate: jax.Array,
    B_w_up: jax.Array,
    B_w_down: jax.Array,
    grad_out: jax.Array,
):
    hbm = pl.BlockSpec(memory_space=pl.ANY)
    sds = jax.ShapeDtypeStruct
    sem = pltpu.SemaphoreType.DMA
    outs = pl.pallas_call(
        _kernel,
        in_specs=[hbm] * 10,
        out_specs=[hbm] * 7,
        out_shape=[sds((D, S), bf16), sds((D, S), bf16), sds((DF, S), bf16), sds((DF, S), bf16),
                   sds((D, F), bf16), sds((D, F), bf16), sds((D, F), bf16)],
        scratch_shapes=[_scratch(k, *v) for k, v in _SCR.items()]
        + [sem((S // CH,)), sem((6,)), sem((6,)), sem((6,))],
        compiler_params=pltpu.CompilerParams(vmem_limit_bytes=127 * 2**20),
        name="gfnet_swiglu_fwdbwd",
    )(A_x.reshape(S, D).T, grad_out.reshape(S, D).T, A_w_r.T, A_w_i.T,
      _DM, _G, _CF, B_w_gate, B_w_up, B_w_down.T)
    out, dx, dwr, dwi, dwg, dwu, dwd = outs
    return (out.T.reshape(1, S, D), dx.T.reshape(1, S, D), dwr.T, dwi.T, dwg, dwu, dwd.T)
```
